```python
import jax
import jax.numpy as jnp

def _softmax(x, axis=-1):
    return jax.nn.softmax(x, axis=axis)
def _gelu(x):
    return jax.nn.gelu(x, approximate=True)
def _silu(x):
    return jax.nn.silu(x)
def _sigmoid(x):
    return jax.nn.sigmoid(x)
def _layernorm(x, axis=-1, eps=1e-5):
    m = jnp.mean(x, axis=axis, keepdims=True)
    v = jnp.var(x, axis=axis, keepdims=True)
    return (x - m) / jnp.sqrt(v + eps)
def _scatter_add(tgt, idx, src, axis=0):
    return tgt.at[idx].add(src)
def _segment_sum(src, seg, n):
    return jax.ops.segment_sum(src, seg, n)
class _Rng:
    def __init__(self, key):
        self._k = key
    def _next(self):
        self._k, sub = jax.random.split(self._k)
        return sub
    def normal(self, shape):
        return jax.random.normal(self._next(), shape, dtype=jnp.bfloat16)
    def randint(self, lo, hi, shape):
        return jax.random.randint(self._next(), shape, lo, hi, dtype=jnp.int32)
    def uniform(self, shape, lo=0.0, hi=1.0):
        return jax.random.uniform(self._next(), shape, jnp.bfloat16, lo, hi)
    def permutation(self, n):
        return jax.random.permutation(self._next(), n)


kernel_name = 'standalone__seq2seq_rnn_t_joint__speech'

def _fwd_setup_inputs():
    _rng = _Rng(jax.random.key(int.from_bytes(__import__("os").urandom(4), "little")))
    _w = (lambda a: (lambda t: t.astype(jnp.bfloat16) if jnp.issubdtype(t.dtype, jnp.floating) else t)(jnp.asarray(a)))
    B, T, D, K = 2, 1000, 512, 5
    U = 8
    sc = (1.0 / (K * D)) ** 0.5
    sd = (1.0 / D) ** 0.5
    return {
        "x": _w((lambda *s: _rng.normal(s) * 0.05)(B, T, D) * 0.5),
        "w1": _w((lambda *s: _rng.normal(s) * 0.05)(K, D, D) * sc),
        "w2": _w((lambda *s: _rng.normal(s) * 0.05)(K, D, D) * sc),
        "g": _w((lambda *s: _rng.normal(s) * 0.05)(B, U, D) * 0.5),
        "w_f": _w((lambda *s: _rng.normal(s) * 0.05)(D, D) * sd),
        "w_g": _w((lambda *s: _rng.normal(s) * 0.05)(D, D) * sd),
        "w_o": _w((lambda *s: _rng.normal(s) * 0.05)(D, D) * sd),
    }

def _fwd_reference(x, w1, w2, g, w_f, w_g, w_o):
    B, T, D = x.shape
    K = w1.shape[0]
    pad = K // 2
    xp = jnp.pad(x, ((0,0),(pad,pad),(0,0)))
    h = jnp.zeros_like(x)
    for i in range(K):
        h = h + jnp.einsum("btc,cd->btd", xp[:, i:i+T, :], w1[i])
    h = _gelu(h)[:, ::2, :]
    T1 = h.shape[1]
    hp = jnp.pad(h, ((0,0),(pad,pad),(0,0)))
    f = jnp.zeros_like(h)
    for i in range(K):
        f = f + jnp.einsum("btc,cd->btd", hp[:, i:i+T1, :], w2[i])
    f = _gelu(f)[:, ::2, :]
    fe = jnp.einsum("btd,de->bte", f, w_f)
    ge = jnp.einsum("bud,de->bue", g, w_g)
    j = jnp.tanh(fe[:, :, None, :] + ge[:, None, :, :])
    return jnp.einsum("btud,dv->btuv", j, w_o)


def setup_inputs():
    _inp = _fwd_setup_inputs()
    _gk = jax.random.fold_in(jax.random.key(int.from_bytes(__import__("os").urandom(4), "little")), 2**31 - 1)
    _shapes = [[2, 250, 8, 512]]
    _dtypes = ['bfloat16']
    _gks = jax.random.split(_gk, len(_shapes))
    _gs = [jax.random.normal(k, s, dtype=jnp.dtype(d)) * 0.05 for k, s, d in zip(_gks, _shapes, _dtypes)]
    _inp["grad_out"] = _gs[0]
    return _inp

def reference(x, w1, w2, g, w_f, w_g, w_o, grad_out):
    _const = dict()
    def _f(*_d):
        return _fwd_reference(**{'x': _d[0], 'w1': _d[1], 'w2': _d[2], 'g': _d[3], 'w_f': _d[4], 'w_g': _d[5], 'w_o': _d[6], **_const})
    _out, _vjp = jax.vjp(_f, x, w1, w2, g, w_f, w_g, w_o)
    _grads = _vjp(grad_out)
    _out0 = jnp.asarray(_out)
    return (_out0, *[jnp.asarray(_g) for _g in _grads])
```

```python
import functools
import math

import jax
import jax.numpy as jnp
import jax.experimental.pallas as pl
import jax.experimental.pallas.tpu as pltpu

F32, BF16, U32 = jnp.float32, jnp.bfloat16, jnp.uint32
B, T, D, U = 2, 1000, 512, 8
T2 = T // 4
R = T2 * U
RP = 2048
NC = D // 128
P = 64
XROWS = 2 * (8 + 8 * P + 8)
JCH = 256
SPAN = 0.85
SPAN2 = 0.95
OFF = 0.4
RATE = 2.5
NG = 62
FLAGS = {"XLA_TPU_RESCHEDULE_DMA_DONES": True}
PLAN_C = [(0, [(0, 1)]), (1, [(1, 1)]), (2, [(2, 1), (3, 1, 0, 1)]), (3, [((1, 0), 1, 1), (4, 1, 0)]),
          (4, [((0, 1), 1, 2), (5, -1, 4)]), (5, [((1, 1), 1, 3)]), (6, [((0, 0), 1, 5)])]
PLAN_DA = [(0, [(0, 1)]), (5, [(1, 1)]), (4, [(2, 1), (3, 1, 0, 1)]), (1, [((1, 0), 1, 1), (4, 1, 0)]),
           (6, [((0, 1), 1, 2), (5, -1, 4)]), (2, [((0, 0), 1, 3)]), (3, [((1, 1), 1, 5)])]
PLAN_DB = [(0, [(0, 1)]), (2, [(1, 1)]), (5, [((0, 1), 1, 1), (2, 1, 0)]), (6, [(3, 1), (4, 1, 0, 1)]),
           (3, [((1, 0), 1, 3), (5, -1, 2)]), (1, [((0, 0), 1, 5)]), (4, [((1, 1), 1, 4)])]
A = math.sqrt(2.0)
GC = math.sqrt(2.0 / math.pi)
GK = 0.044715


def _gelu(x):
    hx = 0.5 * x
    return hx + hx * jnp.tanh(x * (GC + (GC * GK) * (x * x)))


def _gelu_grad(x):
    x2 = x * x
    th = jnp.tanh(x * (GC + (GC * GK) * x2))
    return (0.5 + 0.5 * th) + (x * (1.0 - th * th)) * (0.5 * GC + (1.5 * GC * GK) * x2)


def _in_tf(d):
    hd = 0.5 * d[2]
    ea, oa = d[4] - hd, A * d[3] - (0.5 * A) * d[1]
    eb, ob = d[4] - 2.0 * d[2], (1.0 / A) * d[3] - A * d[1]
    u = [d[0] + (eb - hd), ea + oa, ea - oa, eb + ob, eb - ob]
    if len(d) == 6:
        u.append(d[1] - 2.5 * d[3] + d[5])
    return u


def _in_tf_t(du):
    ea, oa, eb, ob = du[1] + du[2], du[1] - du[2], du[3] + du[4], du[3] - du[4]
    d = [du[0], (-0.5 * A) * oa - A * ob, -2.5 * du[0] - 0.5 * ea - 2.0 * eb,
         A * oa + (1.0 / A) * ob, du[0] + ea + eb]
    if len(du) == 6:
        d[1] = d[1] + du[5]
        d[3] = d[3] - 2.5 * du[5]
        d.append(du[5])
    return d


def _out_tf(m):
    pa, pb = (m[1] + m[2]) * (1.0 / 6.0), (m[3] + m[4]) * (-1.0 / 3.0)
    na, nb = (m[1] - m[2]) * (A / 6.0), (m[3] - m[4]) * (-1.0 / (3.0 * A))
    return [m[0] + pa + pb, na + nb, 2.0 * pa + 0.5 * pb, 2.0 * na + 0.5 * nb + m[5]]


def _out_tf_t(y):
    sa, da = (y[0] + 2.0 * y[2]) * (1.0 / 6.0), (y[1] + 2.0 * y[3]) * (A / 6.0)
    sb, db = (y[0] + 0.5 * y[2]) * (-1.0 / 3.0), (y[1] + 0.5 * y[3]) * (-1.0 / (3.0 * A))
    return [y[0], sa + da, sa - da, sb + db, sb - db, y[3]]


def _fold(a, b, s):
    m = (jax.lax.broadcasted_iota(jnp.int32, a.shape, 0) & s) == 0
    return jnp.where(m, a, b) + pltpu.roll(jnp.where(m, b, a), 8 - s, 0)


def _pk(x):
    return pltpu.bitcast(x.astype(BF16), U32)


def _bf(x):
    return pltpu.bitcast(x, BF16)


def _half(start, n):
    return pl.ds(start // 2, n // 2)


def _str_a(a11, a12, a21, a22):
    return [a11 + a22, a21 + a22, a11, a22, a11 + a12, a21 - a11, a12 - a22]


def _str_b(b11, b12, b21, b22):
    return [b11 + b22, b11, b12 - b22, b21 - b11, b22, b11 + b12, b21 + b22]


def _str_b_t(d):
    return [d[0] + d[1] - d[3] + d[5], d[2] + d[5], d[3] + d[6], d[0] - d[2] + d[4] + d[6]]


def _str_c_t(g11, g12, g21, g22):
    return [g11 + g22, g21 - g22, g12 + g22, g11 + g21, g12 - g11, g22, g11]


def _merge(*lists):
    steps = [(i / len(l), n, i) for n, l in enumerate(lists) for i in range(len(l))]
    return [lists[n][i] for _, n, i in sorted(steps)]


def _kernel(x_hbm, w1_hbm, w2_hbm, g_hbm, wf_hbm, wg_hbm, wo_hbm, go_hbm,
            out_hbm, dx_hbm, dw1_hbm, dw2_hbm, dg_hbm, dwf_hbm, dwg_hbm, dwo_hbm,
            xb, w1b, w2b, gb, wfb, wgb, wob, gob,
            v1, v2, u1, u2, dm1, dm2, gh, gf, fb, fe, dfe, djb, jh, gs, wh, dwh, ma, mb, mj, df, hs, dfw, gq, vq, jq, fq,
            outb, dxb, dw1b, dw2b, dgb, dwfb, dwgb, dwob, isem, osem):
    BP, H = B * P, D // 2
    step = functools.partial
    loads = []

    def load(src, dst):
        cp = pltpu.make_async_copy(src, dst, isem.at[len(loads)])
        cp.start()
        loads.append(cp)
        return cp

    outputs = (out_hbm, dwf_hbm, dg_hbm, dwg_hbm, dw1_hbm, dw2_hbm, dx_hbm, dwo_hbm)

    def store(src, hbm, *idx):
        sem = osem.at[[ref is hbm for ref in outputs].index(True)]
        pltpu.make_async_copy(src, hbm.at[idx] if idx else hbm, sem).start()

    def wait(*cps):
        for cp in cps:
            cp.wait()

    ctx, zero = {"anchor": None, "loading": True}, [0]

    def tied(x):
        if ctx["anchor"] is None:
            return x
        w = pltpu.bitcast(x, U32) if x.dtype == BF16 else x
        y, rounds, sel = ctx["y"], ctx["rounds"], []
        for i in range(0, w.shape[0], 8):
            pos = min(int(ctx["anchor"]), rounds * y.shape[0] // 8 - 1)
            r, c = pos * 8 % y.shape[0], (pos * 8 // y.shape[0] + 1) * y.shape[1] // rounds
            other = y[r:r + 8, c - 128:c]
            other = other if w.dtype == F32 else pltpu.bitcast(other, U32)
            sel.append(jnp.where(ctx["true"], w[i:i + 8], other))
            ctx["anchor"] += 1 / RATE
        w = jnp.concatenate(sel, axis=0)
        return _bf(w) if x.dtype == BF16 else w

    def get(ref, *idx):
        return tied(ref[idx])

    def dot(a, b, ca, cb):
        ctx["y"] = y = jax.lax.dot_general(a, b, (((ca,), (cb,)), ((), ())), preferred_element_type=F32)
        wait(*ctx.pop("wait", ()))
        ctx["rounds"] = max(1, a.shape[ca] // 128 * (y.shape[1] // 128) // 4)
        return y
    _nn, _nt, _tn = (functools.partial(dot, ca=ca, cb=cb) for ca, cb in ((1, 0), (1, 1), (0, 0)))

    def _mix(mxu, *vpu, needs=()):
        ctx["wait"] = needs
        cost = [mm.keywords.get("rows", JCH) for mm in mxu]
        span = (SPAN2 if ctx.get("loading") else SPAN) * sum(cost)
        todo = sorted((span * (i + OFF) / len(l), n, i) for n, l in enumerate(vpu) for i in range(len(l)))
        for k, mm in enumerate(mxu):
            mm()
            while todo and todo[0][0] < sum(cost[:k + 1]):
                at, n, i = todo.pop(0)
                ctx["anchor"] = (at - sum(cost[:k])) / cost[k] * ctx["rounds"] * ctx["y"].shape[0] // 8
                vpu[n][i]()
                ctx["anchor"] = None

    def both(f, r, *args):
        return [jnp.concatenate(x, axis=0) for x in zip(f(r, *args), f(r + 8, *args))]

    def grid(f, rows, cols, *args):
        return [step(f, *args, r, c) for c in cols for r in rows]

    def weight_tf(w, v, r, c):
        e = r + r // 128 * 128
        cs, he, ho = pl.ds(c, 128), _half(e, 16), _half(e + 128, 16)
        raw = [get(w, i, pl.ds(r, 16), cs) for i in range(5)]
        w0, w1, w2, w3, w4 = (x.astype(F32) for x in raw)
        v[0, he, cs] = pltpu.bitcast(raw[0], U32)
        v[0, ho, cs] = pltpu.bitcast(raw[1], U32)
        v[5, he, cs] = pltpu.bitcast(raw[4], U32)
        t, sm = A * w2, w0 + w4
        sa, sb = sm + w4, sm + w0
        for k, val in enumerate((sa + t, sa - t, sb + t, sb - t)):
            v[k + 1, he, cs] = _pk(val)
        t = A * w3
        op, om = w1 + t, w1 - t
        for k, val in enumerate((op, om, op + w1, om + w1)):
            v[k + 1, ho, cs] = _pk(val)

    def put_u(u, r, c, vals):
        for k, val in enumerate(vals):
            u[k % 6, _half(r, 16), pl.ds(2 * c + k // 6 * 128, 128)] = _pk(val)

    def x_tf(r, c):
        def tf(r):
            xw = xb.bitcast(U32)
            w = [get(xw, (r // P) * NC + c // 128, pl.ds(7 + 8 * (r % P) + n, 8, stride=8), slice(None))
                 for n in range(10)]
            even = [pltpu.bitcast(x << 16, F32) for x in w]
            odd = [pltpu.bitcast(x & U32(0xFFFF0000), F32) for x in w[:9]]
            return _in_tf(even[0:6]) + _in_tf(odd[0:5]) + _in_tf(even[4:10]) + _in_tf(odd[4:9])
        vals = both(tf, r)
        put_u(u1, r, c, vals[:11])
        put_u(u1, BP + r, c, vals[11:])

    def conv_fwd(m, u, v, c0):
        def mm(k, rows):
            kn = 256 if k < 5 else 128
            y = _nn(_bf(u[k, :, pl.ds(2 * c0, kn)]), _bf(v[k, _half(2 * c0, kn), :]))
            m[k] = y if c0 == 0 else m[k] + y
        return [step(mm, k, rows=u.shape[1] * (4 if k < 5 else 2)) for k in range(6)]

    def conv_bwd_data(d, dm, v, c0):
        def mm(k, j, rows):
            w = v[k, _half(2 * c0 + j * (128 if k < 5 else 256), 128), :]
            d[k, :, pl.ds(j * 128, 128)] = _nt(_bf(dm[k + zero[(c0 > 0) * 4 + j]]), _bf(w))
        return [step(mm, k, j, rows=2 * dm.shape[1]) for k in range(6) for j in range(4 if k < 5 else 2)]

    def un_tf(d, r, c):
        even = [get(d, k, pl.ds(r, 8), pl.ds(2 * c if k < 5 else c, 128)) for k in range(6)]
        return _in_tf_t(even), _in_tf_t([get(d, k, pl.ds(r, 8), pl.ds(2 * c + 128, 128)) for k in range(5)])

    def conv_bwd_weight(dv, u, dm, c0):
        n = D * BP // (2 * u.shape[1])

        def mm(k, j, rows):
            cols = pl.ds(j * n, n)
            y = _tn(_bf(u[k + zero[j + 2], :, pl.ds(2 * c0, 256 if k < 5 else 128)]),
                    _bf(dm[k + zero[8 + c0 // 128], :, cols]))
            dv[k, :, cols] = y[0:128]
            if k < 5:
                dv[6 + k, :, cols] = y[128:256]
        return [step(mm, k, j, rows=256 if k < 5 else 128) for k in range(6) for j in range(D // n)]

    def dw_post(dv, dw, c0, r, c):
        def tf(r, odd):
            x = [get(dv, 6 * odd + k, pl.ds(r, 8), pl.ds(c, 128)) for k in range(6 - odd)]
            sa, da, sb, db = x[1] + x[2], x[1] - x[2], x[3] + x[4], x[3] - x[4]
            return [x[0] + sa + 2.0 * sb, A * (da + db)] + ([] if odd else [2.0 * sa + sb + x[5]])
        for odd in range(2):
            for i, val in enumerate(both(tf, r, odd)):
                dw[2 * i + odd, pl.ds(c0 + r, 16), pl.ds(c, 128)] = val.astype(BF16)

    def fetch(m, n, r, c):
        return [get(m, k, pl.ds(r, 8), pl.ds(c, 128)) for k in range(n)]

    def in_sequence(x, r):
        if r % P != P - 8:
            return x
        row = jax.lax.broadcasted_iota(jnp.int32, (8, 128), 0) + (P - 8)
        return jnp.where(row * 8 + 4 * (r // BP) < T // 2, x, 0.0)

    def gelu_grad(ref, lead, r, c):
        idx = lead + (pl.ds(r, 8), pl.ds(c, 128))
        d = _gelu_grad(get(ref, *idx))
        ref[idx] = in_sequence(d, r) if lead else d

    def conv1_post(c):
        def act(r, c):
            for q, y in enumerate(_out_tf(fetch(ma, 6, r, c))):
                gh[q, pl.ds(r, 8), pl.ds(c, 128)] = y
                hs[c // 128, 4 * (r // BP) + q, pl.ds(8 + r % BP, 8), :] = in_sequence(_gelu(y), r)

        def tf(r, c):
            h = [get(hs, c // 128, i % 8, pl.ds(8 + r + i // 8, 8), slice(None)) for i in range(-2, 9)]
            return _in_tf(h[0::2]) + _in_tf(h[1::2])
        return (grid(act, range(0, 2 * BP, 8), [c])
                + grid(lambda r, c: put_u(u2, r, c, both(tf, r, c)), range(0, BP, 16), [c]))

    def conv2_post(m, r, c):
        ys = _out_tf(fetch(m, 6, r, c))
        for q in range(4):
            gf[pl.ds(q * BP + r, 8), pl.ds(c, 128)] = ys[q]
        for h in range(2):
            fb[pl.ds(h * BP + r, 8), pl.ds(c, 128)] = pltpu.pack_elementwise(
                [_gelu(ys[2 * h]), _gelu(ys[2 * h + 1])], packed_dtype=BF16)

    def put_dm(dm, r, c, vals):
        for k, val in enumerate(vals):
            dm[k, _half(r, 16), pl.ds(c, 128)] = _pk(val)

    def shifted(d, k, base, r, c, by):
        if 0 <= r + by <= BP - 8:
            return get(d, k, pl.ds(base + r + by, 8), pl.ds(c, 128))
        x = pltpu.roll(get(d, k, pl.ds(base + r, 8), pl.ds(c, 128)), -by % 8, 0)
        return jnp.where(jax.lax.broadcasted_iota(jnp.int32, x.shape, 0) + by >= 0, x, 0.0)

    def dh_post(d, c0, r, c):
        def tf(r):
            e, o = un_tf(d, r, c)
            dh = [e[1] + shifted(d, 5, 0, r, c, -1), o[1], e[2], o[2], e[3], o[3],
                  e[4] + shifted(d, 0, 0, r, 2 * c, 1), o[4] + shifted(d, 0, 0, r, 2 * c + 128, 1)]
            dh = [x * get(gh, i % 4, pl.ds(i // 4 * BP + r, 8), pl.ds(c0 + c, 128)) for i, x in enumerate(dh)]
            return _out_tf_t(dh[:4]) + _out_tf_t(dh[4:])
        vals = both(tf, r)
        put_dm(dm1, r, c0 + c, vals[:6])
        put_dm(dm1, BP + r, c0 + c, vals[6:])

    def dx_post(d, c0, r, c):
        (e0, o0), (e1, o1) = un_tf(d, r, c), un_tf(d, BP + r, c)
        ev = [e0[1] + shifted(d, 5, BP, r, c, -1), e0[2], e0[3], e0[4] + e1[0],
              e1[1] + e0[5], e1[2], e1[3], e1[4] + shifted(d, 0, 0, r, 2 * c, 1)]
        od = [o0[1], o0[2], o0[3], o0[4] + o1[0],
              o1[1], o1[2], o1[3], o1[4] + shifted(d, 0, 0, r, 2 * c + 128, 1)]
        dxw, lc = dxb.bitcast(U32), (c0 + c) // 128
        for i in range(8):
            dxw[r // P * NC + lc, pl.ds(8 * (r % P) + i, 8, stride=8), :] = pltpu.pack_elementwise(
                [ev[i], od[i]], packed_dtype=BF16)
        if r % P == P - 8:
            store(dxb.at[r // P * NC + lc, pl.ds(0, T)], dx_hbm, r // P, slice(None), pl.ds(lc * 128, 128))

    def jrows(s):
        return min(JCH, R - s * JCH)

    def jgrid(f, s, *args):
        return grid(f, range(0, jrows(s), 16), (0, 128), s, *args)

    def load_go(s):
        return [load(go_hbm.at[pl.ds(b * R + s * JCH, jrows(s))], gob.at[b, pl.ds(s * JCH, jrows(s))])
                for b in range(B)]

    def wo_tf(r, c):
        q = [get(wob, pl.ds(i + r, 16), pl.ds(j + c, 128)).astype(F32) for i in (0, H) for j in (0, H)]
        for k, val in enumerate(_str_b(*q)):
            wh[k, _half(r, 16), pl.ds(c, 128)] = _pk(val)

    def go_tf(s, r, c):
        rs = s * JCH + r
        raw = [get(gob, b, pl.ds(rs, 16), pl.ds(j + c, 128)) for b in range(B) for j in (0, H)]
        vals = [_pk(x) for x in _str_c_t(*(x.astype(F32) for x in raw))[:5]]
        for k, val in enumerate(vals + [pltpu.bitcast(raw[3], U32), pltpu.bitcast(raw[0], U32)]):
            gs[k, _half(rs, 16), pl.ds(c, 128)] = val

    def strassen(n, m, plan, product, emit):
        def mm(k, updates, rows):
            y = product(k)
            for dst, sign, *terms in updates:
                val = y
                if terms:
                    part = functools.reduce(lambda a, b: a - b, [mj[t, 0:n, 0:m] for t in terms])
                    val = part + y if sign > 0 else part - y
                if isinstance(dst, tuple):
                    emit(*dst, val)
                else:
                    mj[dst, 0:n, 0:m] = val
        return [step(mm, k, updates, rows=n) for k, updates in plan]

    def factors(tf, src, lead, r0, n, m, dst, raw):
        slot = [k for k in range(7) if k not in raw]
        at = () if len(src.shape) == 2 else (lead,)

        def make(r, c):
            q = [_bf(get(src, *at, pl.ds(r0 + i * n + r, 8), pl.ds(j * m + c, 128))).astype(F32)
                 for i in range(2) for j in range(2)]
            for k, val in enumerate(tf(*q)):
                if k not in raw:
                    dst[lead, slot.index(k), pl.ds(r, 8), pl.ds(c, 128)] = _pk(val)

        def read(k):
            if k in raw:
                return _bf(src[at + (pl.ds(r0 + raw[k] * n, n), pl.ds(raw[k] * m, m))])
            return _bf(dst[lead, slot.index(k)])
        return grid(make, range(0, n, 8), range(0, m, 128)), read

    def dj_mm(s):
        rs = _half(s * JCH, jrows(s))

        def emit(b, j, val):
            djb[b, pl.ds(s * JCH, jrows(s)), pl.ds(j * H, H)] = val
        return strassen(jrows(s), H, PLAN_DA, lambda k: _nt(_bf(gs[k, rs, :]), _bf(wh[k])), emit)

    ge, dge = {}, {}

    def joint(s):
        acc = {}

        def act(c, h, i):
            t, js = s * 32 + 4 * i + 2 * h, []
            for b in range(B):
                for j in (0, H):
                    cs, row, key = pl.ds(j + c, 128), 2 * (h * BP + b * P + s * 8 + i), (b, j + c)
                    if t < T2:
                        th = [jnp.tanh(tied(fe[pl.ds(row + e, 1), cs] + ge[key])) for e in range(2)]
                        dz = [get(djb, b, pl.ds((t + e) * U, U), cs) * (1.0 - th[e] * th[e]) for e in range(2)]
                        js.append(jnp.concatenate(th, axis=0))
                        dge[key] = dge[key] + (dz[0] + dz[1]) if key in dge else dz[0] + dz[1]
                        z = _fold(dz[0], dz[1], 1)
                    else:
                        z = jnp.zeros((U, 128), F32)
                    if i % 2:
                        z = _fold(acc[key, 2], z, 2)
                    if i % 4 == 3:
                        dfe[pl.ds(row - 6, 8), cs] = _fold(acc[key, 4], z, 4)
                    acc[key, 4 if i % 2 else 2] = z
            for k, val in enumerate(_str_a(*js) if js else []):
                jh[k, _half(t * U, 2 * U), pl.ds(c, 128)] = _pk(val)
        return [step(act, c, h, i) for c in (0, 128) for h in range(2) for i in range(8)]

    def out_mm(s):
        rows = pl.ds(s * JCH, jrows(s))

        def emit(b, j, val):
            outb[b, rows, pl.ds(j * H, H)] = val.astype(BF16)
            if j == b:
                store(outb.at[b, rows], out_hbm, pl.ds(b * R + s * JCH, jrows(s)))
        return strassen(jrows(s), H, PLAN_C, lambda k: _nn(_bf(jh[k, _half(s * JCH, jrows(s)), :]), _bf(wh[k])), emit)

    g_tf = [factors(_str_c_t, dm1, k, 0, BP // 2, H, gq, {5: 1, 6: 0}) for k in range(5)]
    v_tf = [[factors(_str_b, v1, k, i * H, H // 2, H, vq.at[i], {1: 0, 4: 1}) for k in range(5)] for i in range(2)]

    def dx_mm(i):
        def component(k):
            def emit(a, b, val):
                ma[k, pl.ds(a * BP, BP), pl.ds(b * H, H)] = val
            return strassen(BP, H, PLAN_DA, lambda q: _nt(g_tf[k][1](q), v_tf[i][k][1](q)), emit)
        return [x for k in range(5) for x in component(k)] + conv_bwd_data(ma, dm1, v1, i * H)[-2:]

    j_tf = [factors(_str_a, jh, k, RP // 4, RP // 8, 128, jq.at[0], {2: 0, 3: 1}) for k in range(7)]
    o_tf = [factors(_str_c_t, gs, k, RP // 4, RP // 8, 128, jq.at[1], {5: 1, 6: 0}) for k in range(7)]

    def dwo_tail(k):
        def emit(a, b, val):
            if k == 4:
                tile = (pl.ds(H + a * 128, 128), pl.ds(H + b * 128, 128))
                dwob[tile] = (df[b, pl.ds(a * 128, 128), :] + val).astype(BF16)
                store(dwob.at[tile], dwo_hbm, *tile)
            else:
                dwh[k, pl.ds(a * 128, 128), pl.ds(b * 128, 128)] += val
        return strassen(128, 128, PLAN_DB, lambda q: _tn(j_tf[k][1](q), o_tf[k][1](q)), emit)

    def dwo_mm(s):
        def mm(k):
            rs = _half(s * JCH, JCH)
            y = _tn(_bf(jh[k, rs, :]), _bf(gs[k, rs, :]))
            dwh[k] = y if s == 0 else dwh[k] + y
        return [step(mm, k) for k in range(7)]

    def dwo_post(i):
        tile = (pl.ds((i // 2) * H, H), pl.ds((i % 2) * H, H))

        def post(r, c):
            val = both(lambda r: _str_b_t(fetch(dwh, 7, r, c)), r)[i]
            if i < 3:
                dwob[pl.ds((i // 2) * H + r, 16), pl.ds((i % 2) * H + c, 128)] = val.astype(BF16)
            else:
                df[c // 128, pl.ds(r, 16), :] = val

        return grid(post, range(0, H, 16), (0, 128)) + [lambda: store(dwob.at[tile], dwo_hbm, *tile)]

    def load_x(i):
        return [load(x_hbm.at[b, :, pl.ds(i * 128, 128)], xb.at[b * NC + i, pl.ds(16, T)]) for b in range(B)]

    def load_w(hbm, buf, i, n):
        ks = pl.ds(i * 128, n * 128)
        return [load(hbm.at[:, ks, :], buf.at[:, ks, :])]

    def k_tf(i):
        return (grid(weight_tf, range(i * 128, i * 128 + 128, 16), range(0, D, 128), w1b, v1),
                grid(x_tf, range(0, BP, 16), [i * 128]))

    def w2_tf(i):
        return grid(weight_tf, range(i * 128, i * 128 + 128, 16), range(0, D, 128), w2b, v2)

    def dj_direct(s):
        def mm(j, b):
            rs, cols = pl.ds(s * JCH, JCH), pl.ds(j * 128, 128)
            djb[b, rs, cols] = _nt(gob[b + zero[j], rs, :], wob[cols, :])
        return grid(mm, range(NC), range(B))

    cp_wo, g00 = load(wo_hbm, wob), load(go_hbm.at[0:JCH], gob.at[0, 0:JCH])
    for i in range(B * NC):
        xb[i, 0:16, :] = jnp.zeros((16, 128), BF16)
        xb[i, 1008:XROWS, :] = jnp.zeros((XROWS - 1008, 128), BF16)
    for k in range(7):
        gs[k, R // 2:RP // 2, :] = jnp.zeros(((RP - R) // 2, H), U32)
        jh[k, R // 2:RP // 2, :] = jnp.zeros(((RP - R) // 2, H), U32)

    def touch(i, carry):
        for ref in (v1, v2, u1, u2, dm1, dm2, gh, gf, fb, fe, dfe, djb, jh, gs, wh, dwh, ma, mb, mj, hs, dfw, df, gq, vq, jq, fq):
            rows = pl.ds(pl.multiple_of(i * 8, 8), 8)
            ref[(0,) * (len(ref.shape) - 2) + (rows, pl.ds(0, 128))] = jnp.zeros((8, 128), ref.dtype)
        return [z - 1 - n for n, z in enumerate(carry)]
    zero += jax.lax.fori_loop(0, 2, touch, [2 + 2 * n for n in range(11)])
    ctx["true"] = zero[1] == 0
    for c in range(NC):
        for i, r in ((6, 0), (7, 0), (0, 8 + BP)):
            hs[c, i, r:r + 8, :] = jnp.zeros((8, 128), F32)
    g01 = load(go_hbm.at[R:R + JCH], gob.at[1, 0:JCH])
    wait(cp_wo, g00)
    g1 = load_go(1)
    d0, d1, d2, d3, c1 = dj_direct(0), dj_direct(1), dj_mm(2), dj_mm(3), conv_fwd(ma, u1, v1, 0)
    _mix(d0[:4], grid(wo_tf, range(0, H, 16), (0, 128)))
    wait(g01)
    g2 = load_go(2)
    _mix(d0[4:], jgrid(go_tf, 0))
    wait(*g1)
    x0, g3, w0 = load_x(0), load_go(3), load_w(w1_hbm, w1b, 0, 1)
    _mix(d1[:3], jgrid(go_tf, 1))
    _mix(d1[3:], jgrid(go_tf, 2), needs=g2)
    _mix(d2[:3], k_tf(0)[1], needs=x0)
    k1 = load_x(1) + load_w(w1_hbm, w1b, 1, 1)
    _mix(d2[3:], jgrid(go_tf, 3), needs=g3)
    k2 = load_x(2) + load_w(w1_hbm, w1b, 2, 1)
    _mix(d3, k_tf(0)[0], needs=w0)
    _mix(c1[:1])
    k3 = load_x(3) + load_w(w1_hbm, w1b, 3, 1)
    _mix(c1[1:], *k_tf(1), needs=k1)
    part1 = load_go(4) + load_w(w2_hbm, w2b, 0, 1)
    _mix(conv_fwd(ma, u1, v1, 128), *k_tf(2), needs=k2)
    part2 = load_go(5) + load_w(w2_hbm, w2b, 1, 2)
    _mix(conv_fwd(ma, u1, v1, 256), *k_tf(3), needs=k3)
    rest = (load_w(w2_hbm, w2b, 3, 1) + load_go(6) + load_go(7)
            + [load(wf_hbm, wfb), load(g_hbm, gb), load(wg_hbm, wgb)])
    _mix(conv_fwd(ma, u1, v1, 384), jgrid(go_tf, 4), w2_tf(0), needs=part1)
    m2 = mb.at[0]
    _mix(dj_mm(4), conv1_post(0), jgrid(go_tf, 5), needs=part2)
    _mix(dj_mm(5) + conv_fwd(m2, u2, v2, 0), conv1_post(128), w2_tf(1) + w2_tf(2)[:16])
    ctx["loading"] = False
    post = conv1_post(256)
    _mix(conv_fwd(m2, u2, v2, 128), post[:16], w2_tf(2)[16:] + jgrid(go_tf, 6), needs=rest)
    _mix(dj_mm(6), post[16:], w2_tf(3))
    _mix(conv_fwd(m2, u2, v2, 256), conv1_post(384))
    _mix(conv_fwd(m2, u2, v2, 384), jgrid(go_tf, 7))
    gev = _nn(gb[...], wgb[...])
    _mix(dj_mm(7), grid(conv2_post, range(0, BP, 8), range(0, D, 128), m2))

    def rows(r, n, j):
        return pl.ds(pl.multiple_of(r + zero[j], 16), n) if j else pl.ds(r, n)

    def fe_mm(groups, lo, n, j, rows):
        cols = pl.ds(j * 128, 128)
        f = [fb[pl.ds(pl.multiple_of(i * P + lo + zero[j], 8), n) if j else pl.ds(i * P + lo, n), :] for i in groups]
        y = _nn(_bf(jnp.concatenate(f, axis=0)), wfb[:, cols])
        for m, i in enumerate(groups):
            fe[pl.ds(2 * (i * P + lo), 2 * n), cols] = y[2 * n * m:2 * n * (m + 1)]
    for b in range(B):
        for c in range(0, D, 128):
            ge[b, c] = gev[b * U:(b + 1) * U, c:c + 128]
    gh_grad = [x for c in range(0, D, 128) for q in range(4) for x in grid(gelu_grad, range(0, 2 * BP, 8), [c], gh, (q,))]
    gf_grad = grid(gelu_grad, range(0, 4 * BP, 8), range(0, D, 128), gf, ())
    dwo = [x for s in range(4) for x in dwo_mm(s)]
    _mix([step(fe_mm, range(4), 0, 8, j, rows=64) for j in (0, 2, 1, 3)])
    _mix([step(fe_mm, g, 8, P - 8, j, rows=224) for g in ((0, 1), (2, 3)) for j in range(NC)], joint(0))
    grads = gf_grad + gh_grad
    for s in range(7):
        _mix(_merge(out_mm(s), dwo[4 * s:4 * s + 4]), joint(s + 1), grads[NG * s:NG * s + NG])
    grads = grads[7 * NG:]

    def df_pack(r, c):
        dfw[_half(r, 16), pl.ds(c, 128)] = _pk(get(dfe, pl.ds(r, 16), pl.ds(c, 128)))

    def df_mm(h, j):
        df[j, pl.ds(h * H, H), :] = _nt(_bf(dfw[rows(h * BP, BP, j), :]), wfb[pl.ds(j * 128, 128), :])

    def df_post(r, c):
        def tf(r):
            return _out_tf_t([get(df, c // 128, pl.ds(2 * (q // 2 * BP + r) + q % 2, 8, stride=2), slice(None))
                              * get(gf, pl.ds(q * BP + r, 8), pl.ds(c, 128)) for q in range(4)])
        put_dm(dm2, r, c, both(tf, r))

    def dwf_emit(a, b, val):
        dwfb[pl.ds(a * H, H), pl.ds(b * H, H)] = val.astype(BF16)
    f_tf, f_get = factors(_str_a, fb, 0, 0, BP, H, fq, {2: 0, 3: 1})
    d_tf, d_get = factors(_str_c_t, dfw, 1, 0, BP, H, fq, {5: 1, 6: 0})
    _mix(out_mm(7), grid(df_pack, range(0, D, 16), range(0, D, 128)), f_tf + grads[:NG + 20])
    _mix(grid(df_mm, range(2), range(NC)), grads[NG + 20:2 * NG], d_tf + j_tf[2][0] + o_tf[2][0])
    dge16 = jnp.concatenate([jnp.concatenate([dge[b, c] for c in range(0, D, 128)], axis=1)
                             for b in range(B)], axis=0).astype(BF16)
    dgb[...] = _nt(dge16, wgb[...]).astype(BF16)

    def dwg_mm(rows):
        dwgb[...] = _tn(gb[...], dge16).astype(BF16)
    _mix(strassen(H, H, PLAN_DB, lambda q: _tn(f_get(q), d_get(q)), dwf_emit) + [step(dwg_mm, rows=D)],
         grid(df_post, range(0, BP, 16), range(0, D, 128)), grads[2 * NG:])
    store(dwfb, dwf_hbm)
    store(dgb, dg_hbm)
    store(dwgb, dwg_hbm)

    def dw_grid(i, dw, hbm, c0):
        rows = pl.ds(c0, 128)
        return (grid(dw_post, range(0, 128, 16), range(0, D, 128), mb.at[i], dw, c0)
                + [lambda: store(dw.at[:, rows, :], hbm, slice(None), rows, slice(None))])

    def half(f, d, c0):
        return grid(f, range(0, BP, 16 if f is dh_post else 8), (0, 128), d, c0)

    def tail_tf(*ks):
        return [x for k in ks for x in j_tf[k][0] + o_tf[k][0]]

    def weights(i, u, dm, c0):
        return conv_bwd_weight(mb.at[i], u, dm, c0) + conv_bwd_weight(mb.at[i + 1], u, dm, c0 + 128)

    def weights_post(i, dw, hbm, c0):
        return dw_grid(i, dw, hbm, c0) + dw_grid(i + 1, dw, hbm, c0 + 128)
    va, vb, gt = ([x for steps, _ in v for x in steps] for v in v_tf + [g_tf])
    _mix(conv_bwd_data(mb.at[0], dm2, v2, 0), tail_tf(5) + va[:80])
    _mix(conv_bwd_data(mb.at[1], dm2, v2, H) + dwo_tail(2), half(dh_post, mb.at[0], 0), va[80:100])
    _mix(weights(2, u2, dm2, 0) + dwo_tail(5), half(dh_post, mb.at[1], H), va[100:120])
    _mix(weights(0, u1, dm1, 0), weights_post(2, dw2b, dw2_hbm, 0), gt + tail_tf(6))
    _mix(weights(2, u1, dm1, H), weights_post(0, dw1b, dw1_hbm, 0), va[120:] + vb[:30] + tail_tf(0))
    _mix(dx_mm(0), weights_post(2, dw1b, dw1_hbm, H), vb[30:80] + tail_tf(3))
    _mix(weights(0, u2, dm2, H) + dwo_tail(6), half(dx_post, ma, 0), vb[80:])
    _mix(dx_mm(1), weights_post(0, dw2b, dw2_hbm, H), tail_tf(1, 4))
    q11, q12, q21, q22 = (dwo_post(i) for i in range(4))
    _mix(dwo_tail(0) + dwo_tail(3), half(dx_post, ma, H))
    _mix(dwo_tail(1), q22[:-1] + q12 + q21)
    _mix(dwo_tail(4), q11)
    for i, hbm in enumerate(outputs):
        pltpu.make_async_copy(hbm, hbm, osem.at[i]).wait()


@jax.jit
def pallas_standalone__seq2seq_rnn_t_joint__speech_kernel(
    x: jax.Array,
    w1: jax.Array,
    w2: jax.Array,
    g: jax.Array,
    w_f: jax.Array,
    w_g: jax.Array,
    w_o: jax.Array,
    grad_out: jax.Array,
):
    assert x.shape == (B, T, D) and w1.shape == (5, D, D) and g.shape == (B, U, D)
    vm = pltpu.VMEM
    mat, taps = vm((D, D), BF16), vm((5, D, D), BF16)
    scratch = [
        vm((B * NC, XROWS, 128), BF16), taps, taps, vm((B * U, D), BF16), mat, mat, mat,
        vm((B, RP, D), BF16),
        vm((6, D, D), U32), vm((6, D, D), U32),
        vm((6, B * P, 2 * D), U32), vm((6, B * P // 2, 2 * D), U32),
        vm((6, B * P, D), U32), vm((6, B * P // 2, D), U32),
        vm((4, 2 * B * P, D), F32), vm((4 * B * P, D), F32),
        vm((2 * B * P, D), U32), vm((4 * B * P, D), F32), vm((4 * B * P, D), F32),
        vm((B, RP, D), F32), vm((7, RP // 2, D // 2), U32), vm((7, RP // 2, D // 2), U32),
        vm((7, D // 4, D // 2), U32), vm((7, D // 2, D // 2), F32),
        vm((6, 2 * B * P, D), F32), vm((4, 11, B * P, D), F32), vm((6, JCH, D // 2), F32),
        vm((NC, 4 * B * P + 8, 128), F32), vm((NC, 8, B * P + 16, 128), F32),
        vm((D // 2, D), U32), vm((5, 5, B * P // 2, D // 2), U32),
        vm((2, 5, 5, D // 4, D // 2), U32), vm((2, 7, 5, RP // 8, 128), U32),
        vm((2, 5, B * P, D // 2), U32),
        vm((B, RP, D), BF16), vm((B * NC, 16 * P + 16, 128), BF16),
        taps, taps,
        vm((B * U, D), BF16), mat, mat, mat,
        pltpu.SemaphoreType.DMA((40,)), pltpu.SemaphoreType.DMA((8,)),
    ]
    sds = jax.ShapeDtypeStruct
    out_shape = [sds((B * R, D), BF16), sds(x.shape, BF16), sds(w1.shape, BF16), sds(w2.shape, BF16),
                 sds((B * U, D), BF16), sds((D, D), BF16), sds((D, D), BF16), sds((D, D), BF16)]
    hbm = pl.BlockSpec(memory_space=pl.ANY)
    out, dx, dw1, dw2, dg, dwf, dwg, dwo = pl.pallas_call(
        _kernel,
        in_specs=[hbm] * 8,
        out_specs=[hbm] * 8,
        out_shape=out_shape,
        scratch_shapes=scratch,
        compiler_params=pltpu.CompilerParams(vmem_limit_bytes=124 * 1024 * 1024, flags=FLAGS),
    )(x, w1, w2, g.reshape(B * U, D), w_f, w_g, w_o, grad_out.reshape(B * R, D))
    return (out.reshape(B, T2, U, D), dx, dw1, dw2, dg.reshape(B, U, D), dwf, dwg, dwo)
```
